```python
import os as _os
_os.environ.setdefault("JAX_PLATFORMS", "cpu")
import jax
import jax.numpy as jnp

def _softmax(x, axis=-1):
    return jax.nn.softmax(x, axis=axis)
def _gelu(x):
    return jax.nn.gelu(x, approximate=True)
def _silu(x):
    return jax.nn.silu(x)
def _sigmoid(x):
    return jax.nn.sigmoid(x)
def _layernorm(x, axis=-1, eps=1e-5):
    m = jnp.mean(x, axis=axis, keepdims=True)
    v = jnp.var(x, axis=axis, keepdims=True)
    return (x - m) / jnp.sqrt(v + eps)
def _scatter_add(tgt, idx, src, axis=0):
    return tgt.at[idx].add(src)
def _segment_sum(src, seg, n):
    return jax.ops.segment_sum(src, seg, n)
class _Rng:
    def __init__(self, key):
        self._k = key
    def _next(self):
        self._k, sub = jax.random.split(self._k)
        return sub
    def normal(self, shape):
        return jax.random.normal(self._next(), shape, dtype=jnp.bfloat16)
    def randint(self, lo, hi, shape):
        return jax.random.randint(self._next(), shape, lo, hi, dtype=jnp.int32)
    def uniform(self, shape, lo=0.0, hi=1.0):
        return jax.random.uniform(self._next(), shape, jnp.bfloat16, lo, hi)
    def permutation(self, n):
        return jax.random.permutation(self._next(), n)


kernel_name = 'parallel_sum__sliding_local_dilated__geglu_ffn__prompt'

def setup_inputs():
    _rng = _Rng(jax.random.key(int.from_bytes(__import__("os").urandom(4), "little")))
    _w = (lambda a: (lambda t: t.astype(jnp.bfloat16) if jnp.issubdtype(t.dtype, jnp.floating) else t)(jnp.asarray(a)))
    def _A_setup():
        B, S, D = 1, 2048, 640
        return {
            "x": _w((lambda *s: _rng.normal(s) * 0.05)(B, S, D)),
            "wqkv": _w((lambda *s: _rng.normal(s) * 0.05)(D, 3 * D)),
            "wo": _w((lambda *s: _rng.normal(s) * 0.05)(D, D)),
        }
    _A_in = _A_setup()

    def _B_setup():
        B, S, D, F = 1, 2048, 640, 1728
        return {
            "x": _w((lambda *s: _rng.normal(s) * 0.05)(B, S, D)),
            "w_gate": _w((lambda *s: _rng.normal(s) * 0.05)(D, F)),
            "w_up": _w((lambda *s: _rng.normal(s) * 0.05)(D, F)),
            "w_down": _w((lambda *s: _rng.normal(s) * 0.05)(F, D)),
        }
    _B_in = _B_setup()

    return {
        "A_x": _A_in["x"],
        "A_wqkv": _A_in["wqkv"],
        "A_wo": _A_in["wo"],
        "B_x": _B_in["x"],
        "B_w_gate": _B_in["w_gate"],
        "B_w_up": _B_in["w_up"],
        "B_w_down": _B_in["w_down"],
    }

def reference(A_x, A_wqkv, A_wo, B_x, B_w_gate, B_w_up, B_w_down):
    def _A_ref(x, wqkv, wo):
        B, S, D = x.shape
        H = 32; Dh = D // H
        W, dil = 8, 2
        qkv = (lambda x, *d: x.transpose(*d))((x @ wqkv).reshape(B, S, 3, H, Dh), 2, 0, 3, 1, 4)
        q, k, v = qkv[0], qkv[1], qkv[2]
        scale = Dh ** -0.5
        pos = jnp.arange(S)
        off = jnp.arange(W) * dil
        idx = pos[:, None] - off[None, :]
        mask = idx >= 0
        idx_c = jnp.where(mask, idx, 0).reshape(-1)
        kg = k[:, :, idx_c, :].reshape(B, H, S, W, Dh)
        vg = v[:, :, idx_c, :].reshape(B, H, S, W, Dh)
        logits = jnp.einsum("bhsd,bhswd->bhsw", q, kg) * scale
        logits = jnp.where(mask[None, None, :, :], logits, -1e9)
        attn = _softmax(logits, axis=-1)
        o = jnp.einsum("bhsw,bhswd->bhsd", attn, vg)
        return (lambda x, *d: x.transpose(*d))(o, 0, 2, 1, 3).reshape(B, S, D) @ wo

    def _B_ref(x, w_gate, w_up, w_down):
        return (_gelu(x @ w_gate) * (x @ w_up)) @ w_down

    x = A_x
    xn = _layernorm(x, axis=-1)
    return x + _A_ref(xn, A_wqkv, A_wo) + _B_ref(xn, B_w_gate, B_w_up, B_w_down)
```

```python
import functools, os
import jax
import jax.numpy as jnp
from jax import lax
import jax.experimental.pallas as pl
import jax.experimental.pallas.tpu as pltpu

E = lambda k, d: int(os.environ.get('KP_' + k, d))
TM0 = E('TM0', 512)
TM = E('TM', 384)
RC = E('RC', 8)
LR = E('LR', 32)
LGAP = E('LGAP', 4)
PLEAD = E('PLEAD', 2)
PGAP = E('PGAP', 2)
AGAP0 = E('AGAP0', 0)
AGAP = E('AGAP', 0)
AM = E('AM', 128)
NFIRST = E('NFIRST', 6)
SCOPES = E('SCOPES', 0)
FC = 128
LR0 = E('LR0', 64)
WGAP = E('WGAP', 2)
NXP = E('NXP', 2)
H, DH, W, DIL = 32, 20, 8, 2
HALO = 16
S = 2048
D = 640
F = 1728
NT = D // 128
FMAIN = (F // 128) * 128
NCH = FMAIN // FC
FP = FMAIN + 128
NB = 1 + (S - TM0) // TM
TMX = max(TM, TM0)
NTDIMS = (((1,), (1,)), ((), ()))
f32 = jnp.float32
bf16 = jnp.bfloat16
u32 = jnp.uint32


def _pk(v):
    return pltpu.bitcast(v.astype(bf16), u32)


def _upk(v):
    return pltpu.bitcast(v, bf16)

OSPLIT = [int(v) for v in os.environ.get('KP_OSPLIT', '0,128,256,384,512,640').split(',')]


def _gelu(g):
    c = 0.7978845608028654
    return 0.5 * g * (1.0 + jnp.tanh(c * (g + 0.044715 * (g * g * g))))


def _ln(ref, rows):
    x = [ref[rows, t * 128:(t + 1) * 128].astype(f32) for t in range(NT)]
    mu = jnp.sum(sum(x[1:], x[0]), axis=-1, keepdims=True) * (1.0 / D)
    xc = [v - mu for v in x]
    sq = [v * v for v in xc]
    var = jnp.sum(sum(sq[1:], sq[0]), axis=-1, keepdims=True) * (1.0 / D)
    r = lax.rsqrt(var + 1e-5)
    return [_pk(v * r) for v in xc]


def _spread(items, n):
    k, r = divmod(len(items), n)
    out, p = [], 0
    for j in range(n):
        m = k + (1 if j < r else 0)
        out.append(items[p:p + m])
        p += m
    return out


def kernel(x_hbm, wqkv_hbm, wo_hbm, wg_hbm, wu_hbm, wd_hbm, o_hbm,
           x_sc, xn_sc, q_sc, kv_sc, a_sc, h_sc, o_sc, wg_sc, wu_sc, wt_sc, wo_sc, wd_sc,
           wqkv_raw, wq_sc, wk_sc, wv_sc, wo_raw, tr_sc, sems, osem):
    i = pl.program_id(0)
    z = lax.shift_right_logical(i, 20)
    z16 = pl.multiple_of(z * 16, 16)
    scale = DH ** -0.5 * 1.4426950408889634
    wp_sc = (wq_sc, wk_sc, wv_sc)

    copies = {}
    def mk(name, src, dst):
        copies[name] = pltpu.make_async_copy(src, dst, sems.at[len(copies)])
    def mk_gu(c0, c1):
        mk('g%d' % c0, wg_hbm.at[c0 * FC:c1 * FC, :], wg_sc.at[c0 * FC:c1 * FC, :])
        mk('u%d' % c0, wu_hbm.at[c0 * FC:c1 * FC, :], wu_sc.at[c0 * FC:c1 * FC, :])
    def mk_qkv(s):
        mk('qkv%d' % s, wqkv_hbm.at[:, s * D:(s + 1) * D], wqkv_raw.at[0:D, s * D:(s + 1) * D])
    XP = TM0 // NXP
    for j in range(NXP):
        mk('x0%d' % j, x_hbm.at[j * XP:(j + 1) * XP, :], x_sc.at[j * XP:(j + 1) * XP, :])
    mk_gu(0, 1)
    mk_gu(1, 3)
    mk_gu(3, 7)
    mk_qkv(0)
    mk_qkv(1)
    mk_gu(7, 10)
    mk_qkv(2)
    mk_gu(10, NCH)
    mk('wo', wo_hbm, wo_raw.at[0:D, :])
    mk('gt', wg_hbm.at[FMAIN:F, :], wt_sc.at[0:64, :])
    mk('ut', wu_hbm.at[FMAIN:F, :], wt_sc.at[64:128, :])
    mk('x1', x_hbm.at[TM0:TM0 + TM, :], x_sc.at[TM0:TM0 + TM, :])
    mk('wd', wd_hbm, wd_sc.at[0:F, :])
    mk('xr', x_hbm.at[TM0 + TM:S, :], x_sc.at[TM0 + TM:S, :])

    def wait(*names):
        for n in names:
            if SCOPES:
                with jax.named_scope('wait_' + n):
                    copies[n].wait()
            else:
                copies[n].wait()

    def tok(ref):
        v = ref[pl.ds(z16, 16), 0:128]
        return _upk(v)[0:16] if v.dtype == u32 else v

    def before(ref, val):
        n = ref.shape[0]
        v = val[0:16, 0:128].astype(bf16)
        if ref.dtype == u32:
            ref[pl.ds(n - 16 + z16, 8), 0:128] = pltpu.bitcast(v, u32)
        else:
            ref[pl.ds(n - 16 + z16, 16), 0:128] = v

    def before_q(val):
        q_sc[NT + z, 0:8, :] = val[0:8, 0:128]

    def run(units, pieces):
        due = {}
        def emit(k, r):
            for su, srow, fence, thunk, du in pieces:
                if su == k:
                    if r is not None:
                        fence(r[srow:srow + 16])
                    t = thunk()
                    if du is not None and du < len(units):
                        due[du] = due.get(du, []) + [t()]
        emit(-1, None)
        for k, (ref, thunk) in enumerate(units):
            for t in due.get(k, []):
                before(ref, t)
            emit(k, thunk())

    def gather(slot, dst, t):
        for d in range(DH):
            dst[d * H // 2:(d + 1) * H // 2, t * 128:(t + 1) * 128] = _pk(tr_sc[slot, pl.ds(d, H, stride=DH), :])
        return lambda: tok(dst)

    def perm_qkv(s, t):
        slot = t % 2
        for j in range(NT):
            blk = wqkv_raw[t * 128:(t + 1) * 128, s * D + j * 128:s * D + (j + 1) * 128].astype(f32)
            tr_sc[slot, j * 128:(j + 1) * 128, :] = blk.T
        return gather(slot, wp_sc[s], t)

    def perm_wo(t):
        slot = t % 2
        tr_sc[slot] = wo_raw[0:D, t * 128:(t + 1) * 128].astype(f32)
        return gather(slot, wo_sc, t)

    def proj_tile(xn, n):
        tm = xn.shape[0]
        s, t = divmod(n, NT)
        w = _upk(wp_sc[s][t * 64:(t + 1) * 64, :])
        r = lax.dot_general(xn, w, NTDIMS, preferred_element_type=f32)
        if n < NT:
            q_sc[n, 0:tm, :] = r * scale
        else:
            kv_sc[n - NT, HALO:HALO + tm, :] = r
        return r

    def ln_rows(nxt, rr):
        for r0 in rr:
            for t, v in enumerate(_ln(x_sc, pl.ds(pl.multiple_of(nxt + r0, 16), LR))):
                xn_sc[r0 // 2:(r0 + LR) // 2, t * 128:(t + 1) * 128] = v
        return lambda: tok(xn_sc)

    def attn(r0, first):
        q = [q_sc[t, r0:r0 + RC, :] for t in range(NT)]
        logits = []
        for w in range(W):
            off = r0 + HALO - w * DIL
            s = q[0] * kv_sc[0, off:off + RC, :]
            for t in range(1, NT):
                s = s + q[t] * kv_sc[t, off:off + RC, :]
            s = s + pltpu.roll(s, 64, 1)
            s = s + pltpu.roll(s, 32, 1)
            if first and w > 0 and r0 < HALO:
                pos = r0 + lax.broadcasted_iota(jnp.int32, (RC, 128), 0)
                s = jnp.where(pos >= w * DIL, s, -1e9)
            logits.append(s)
        m = logits[0]
        for w in range(1, W):
            m = jnp.maximum(m, logits[w])
        p = [jnp.exp2(l - m) for l in logits]
        den = p[0]
        for w in range(1, W):
            den = den + p[w]
        inv = pl.reciprocal(den, approx=True)
        for t in range(NT):
            acc = p[0] * kv_sc[NT + t, r0 + HALO:r0 + HALO + RC, :]
            for w in range(1, W):
                off = r0 + HALO - w * DIL
                acc = acc + p[w] * kv_sc[NT + t, off:off + RC, :]
            a_sc[r0:r0 + RC, t * 128:(t + 1) * 128] = (acc * inv).astype(bf16)

    def attn_rows(rr, first):
        for r0 in rr:
            attn(r0, first)
        return lambda: tok(a_sc)

    def attn_pieces(tm, u0, u1, gap, first):
        nm = max(1, tm // AM)
        slots = [(u, k * (tm // nm)) for u in range(u0, u1) for k in range(nm if u >= 0 else 1)]
        rows = list(range(0, tm, RC))
        n = len(rows)
        out = []
        for j, (u, srow) in enumerate(slots):
            rr = rows[-(-j * n // len(slots)):-(-(j + 1) * n // len(slots))]
            if rr:
                last = j + 1 == len(slots) or slots[j + 1][0] != u
                out.append((u, srow, before_q, functools.partial(attn_rows, rr, first),
                            u + gap if (gap and last) else None))
        return out

    def dot_nt(x, w, split=1):
        m = x.shape[0] // split
        parts = [lax.dot_general(x[k * m:(k + 1) * m], w, NTDIMS, preferred_element_type=f32) for k in range(split)]
        return parts[0] if split == 1 else jnp.concatenate(parts, axis=0)

    class Ffn:
        def __init__(self, xn):
            self.xn, self.g, self.h = xn, {}, {}
        def gate(self, c, split=1):
            self.g[c] = dot_nt(self.xn, wg_sc[c * FC:(c + 1) * FC, :], split)
            return self.g[c]
        def up(self, c, split=1):
            u = dot_nt(self.xn, wu_sc[c * FC:(c + 1) * FC, :], split)
            h_sc[0:u.shape[0] // 2, c * FC:(c + 1) * FC] = _pk(_gelu(self.g[c]) * u)
            return u
        def tail(self, split=1):
            gu = dot_nt(self.xn, wt_sc[0:128, :], split)
            h = _gelu(gu) * pltpu.roll(gu, 64, 1)
            lane = lax.broadcasted_iota(jnp.int32, gu.shape, 1)
            h_sc[0:gu.shape[0] // 2, FMAIN:FP] = _pk(jnp.where(lane < 64, h, 0.0))
            return gu
        def G(self, c, split=1): return (wg_sc, functools.partial(self.gate, c, split))
        def U(self, c, split=1): return (wu_sc, functools.partial(self.up, c, split))
        def GU(self, *cs): return [x for c in cs for x in (self.G(c), self.U(c))]
        def T(self, split=1): return (wt_sc, functools.partial(self.tail, split))
        def P(self, *ns): return [(wp_sc[n // NT], functools.partial(proj_tile, self.xn, n)) for n in ns]

    def emit_out(row0, tm, n0, n1, y):
        o_sc[pl.ds(row0, tm), n0:n1] = (x_sc[pl.ds(row0, tm), n0:n1].astype(f32) + y).astype(bf16)
        pltpu.make_async_copy(o_sc.at[pl.ds(row0, tm), n0:n1], o_hbm.at[pl.ds(row0, tm), n0:n1], osem).start()

    def halo(tm):
        kv_sc[:, 0:HALO, :] = kv_sc[:, tm:tm + HALO, :]

    lrows = list(range(0, TM, LR))
    bx = functools.partial(before, x_sc)

    @pl.when(i == 0)
    def _():
        names = list(copies)
        for n in names[:NFIRST]:
            copies[n].start()
        kv_sc[:, 0:HALO, :] = jnp.zeros((2 * NT, HALO, 128), f32)
        wd_sc[F:FP, :] = jnp.zeros((FP - F, D), bf16)
        xs = []
        for j in range(NXP):
            wait('x0%d' % j)
            if j == 0:
                for n in names[NFIRST:]:
                    copies[n].start()
            for r0 in range(j * XP, (j + 1) * XP, LR0):
                for t, v in enumerate(_ln(x_sc, pl.ds(r0, LR0))):
                    xn_sc[r0 // 2:(r0 + LR0) // 2, t * 128:(t + 1) * 128] = v
        wait('g0', 'u0')
        f = Ffn(_upk(xn_sc[0:TM0 // 2, :]))
        run([f.G(0, 2), f.U(0, 2)], [])
        wait('g1', 'u1')
        run(f.GU(1, 2), [])
        wait('g3', 'u3')
        run(f.GU(3, 4, 5, 6), [])

        def perm_pieces(thunks):
            return [(max(j - PLEAD, -1), 0, functools.partial(before, src), th, j + PGAP)
                    for j, (src, th) in enumerate(thunks)]
        pq = lambda s: [(wqkv_raw, functools.partial(perm_qkv, s, t)) for t in range(NT)]
        wait('qkv0', 'qkv1', 'g7', 'u7')
        run(f.GU(7, 8, 9) + f.P(*range(10)), perm_pieces(pq(0) + pq(1)))
        wait('qkv2', 'g10', 'u10', 'wo', 'gt', 'ut', 'x1', 'wd')

        st = {}
        KH = FP // 2
        def down(n, half):
            y = jnp.dot(_upk(h_sc[0:TM0 // 2, half * KH:(half + 1) * KH]), wd_sc[half * KH:(half + 1) * KH, n * 128:(n + 1) * 128],
                        preferred_element_type=f32)
            st[n] = y if half == 0 else st[n] + y
            return y
        def oproj(n):
            if 'a' not in st:
                halo(TM0)
                st['a'] = a_sc[0:TM0, :]
            split = 4 if n == NT - 1 else 1
            m = TM0 // split
            w = _upk(wo_sc[0:D // 2, n * 128:(n + 1) * 128])
            y = jnp.concatenate([jnp.dot(st['a'][k * m:(k + 1) * m], w, preferred_element_type=f32) for k in range(split)], axis=0)
            emit_out(0, TM0, n * 128, (n + 1) * 128, st[n] + y)
            return y
        units = (f.GU(10, 11) + f.GU(12) + f.P(*range(10, 15)) + [f.T()]
                 + [(wd_sc, functools.partial(down, n, half)) for n in range(NT) for half in range(2)]
                 + [(wo_sc, functools.partial(oproj, n)) for n in range(NT)])
        pieces = perm_pieces(pq(2))
        pieces += [(5 + t - PLEAD, 0, functools.partial(before, wo_raw), functools.partial(perm_wo, t), 5 + t + WGAP) for t in range(NT)]
        pieces += [(j, 256, bx, functools.partial(ln_rows, TM0 + z16, rr), j + 3) for j, rr in enumerate(_spread(lrows, 8))]
        pieces += attn_pieces(TM0, 11, E('A0END', 21), AGAP0, True)
        run(units, pieces)
        wait('xr')

    @pl.when(i > 0)
    def _():
        row0 = pl.multiple_of(TM0 + (i - 1) * TM, 16)
        nxt = jnp.minimum(row0 + TM, S - TM)
        f = Ffn(_upk(xn_sc[0:TM // 2, :]))
        units = f.P(*range(15)) + f.GU(*range(NCH)) + [f.T()]
        pieces = [(j, 0, bx, functools.partial(ln_rows, nxt, rr), j + LGAP)
                  for j, rr in enumerate(_spread(lrows, min(len(lrows), 15 - LGAP)))]
        pieces += attn_pieces(TM, 15, 15 + 2 * NCH, AGAP, False)
        run(units, pieces)
        halo(TM)
        a = a_sc[0:TM, :]
        for j in range(len(OSPLIT) - 1):
            n0, n1 = OSPLIT[j], OSPLIT[j + 1]
            lhs = jnp.concatenate([a, _upk(h_sc[0:TM // 2, :])], axis=1)
            wo_ = _upk(wo_sc[0:D // 2, n0:n1])
            rhs = jnp.concatenate([wo_, wd_sc[0:FP, n0:n1]], axis=0)
            emit_out(row0, TM, n0, n1, jnp.dot(lhs, rhs, preferred_element_type=f32))

    @pl.when(i == NB - 1)
    def _():
        pltpu.make_async_copy(o_sc, o_hbm, osem).wait()


@jax.jit
def pallas_parallel_sum__sliding_local_dilated__geglu_ffn__prompt_kernel(A_x, A_wqkv, A_wo, B_x, B_w_gate, B_w_up, B_w_down):
    B = A_x.shape[0]
    x = A_x.reshape(S, D)
    anyspec = pl.BlockSpec(memory_space=pl.ANY)
    out = pl.pallas_call(
        kernel,
        grid=(NB,),
        in_specs=[anyspec] * 6,
        out_specs=anyspec,
        out_shape=jax.ShapeDtypeStruct((S, D), A_x.dtype),
        scratch_shapes=[pltpu.VMEM((S + 16, D), bf16),
                        pltpu.VMEM((TMX // 2, D), u32),
                        pltpu.VMEM((NT + 1, TMX, 128), f32),
                        pltpu.VMEM((2 * NT, TMX + HALO, 128), f32),
                        pltpu.VMEM((TMX, D), bf16),
                        pltpu.VMEM((TMX // 2, FP), u32),
                        pltpu.VMEM((S, D), bf16),
                        pltpu.VMEM((FMAIN + 16, D), bf16),
                        pltpu.VMEM((FMAIN + 16, D), bf16),
                        pltpu.VMEM((128 + 16, D), bf16),
                        pltpu.VMEM((D // 2 + 16, D), u32),
                        pltpu.VMEM((FP + 16, D), bf16),
                        pltpu.VMEM((D + 16, 3 * D), bf16),
                        pltpu.VMEM((D // 2 + 16, D), u32),
                        pltpu.VMEM((D // 2 + 16, D), u32),
                        pltpu.VMEM((D // 2 + 16, D), u32),
                        pltpu.VMEM((D + 16, D), bf16),
                        pltpu.VMEM((2, D, 128), f32),
                        pltpu.SemaphoreType.DMA((24,)),
                        pltpu.SemaphoreType.DMA(()),
                        ],
        compiler_params=pltpu.CompilerParams(dimension_semantics=("arbitrary",), vmem_limit_bytes=100 * 1024 * 1024,
                                             disable_semaphore_checks=True, disable_bounds_checks=True),
    )(x, A_wqkv, A_wo, B_w_gate.T, B_w_up.T, B_w_down)
    return out.reshape(B, S, D)
```

```python
import functools

import jax
import jax.numpy as jnp
from jax import lax
import jax.experimental.pallas as pl
import jax.experimental.pallas.tpu as pltpu

S, D, F = 2048, 640, 1728
H, DH, W, DIL = 32, 20, 8, 2
HALO = 16
TM0 = 512
TM = 384
NB = 1 + (S - TM0) // TM
TMX = max(TM, TM0)
HT, HM = TM0 // 2, TM // 2
NT = D // 128
FC = 128
FMAIN = (F // FC) * FC
NCH = FMAIN // FC
FP = FMAIN + 128
RC = 8
LR = 16
KS = 256
NKH = (NCH + 1) // 2
NKP = NKH + 2
KD = NKP * 128
PAIRS = ([(('p', a), ('p', a + 1)) for a in (0, 2, 5, 7, 10, 12)] + [(('p', 4), ('p', 9))]
         + [((m, c), (m, c + 1)) for c in range(0, 12, 2) for m in 'gu'])
NT_DIMS = (((1,), (1,)), ((), ()))
NN_DIMS = (((1,), (0,)), ((), ()))
f32, bf16, u32 = jnp.float32, jnp.bfloat16, jnp.uint32


def _pk(v):
    return pltpu.bitcast(v.astype(bf16), u32)


def _upk(v):
    return pltpu.bitcast(v, bf16)


def _gelu(g):
    c = 0.7978845608028654
    return 0.5 * g * (1.0 + jnp.tanh(c * (g + 0.044715 * (g * g * g))))


def _ln(ref, rows):
    x = [ref[rows, t * 128:(t + 1) * 128].astype(f32) for t in range(NT)]
    mu = jnp.sum(sum(x[1:], x[0]), axis=-1, keepdims=True) * (1.0 / D)
    mb = mu.astype(bf16).astype(f32)
    xc = [v - mb for v in x]
    sq = [v * v for v in xc]
    var = jnp.sum(sum(sq[1:], sq[0]), axis=-1, keepdims=True) * (1.0 / D) - (mu - mb) * (mu - mb)
    r = lax.rsqrt(jnp.maximum(var, 0.0) + 1e-5)
    return [v * r for v in xc]


def _lcomb(a11, a12, a21, a22):
    return a11 + a22, a21 + a22, a11 + a12, a21 - a11, a12 - a22


def _rcomb(b11, b12, b21, b22):
    return b11 + b22, b12 - b22, b21 - b11, b11 + b12, b21 + b22


def _ocomb(m):
    return (jnp.concatenate([(m[4] - m[5]) + (m[1] + m[7]), m[4] + m[2]], axis=0),
            jnp.concatenate([m[5] + m[3], (m[1] + (m[3] - m[2])) + m[6]], axis=0))


def _dot(x, w, dims, split=1):
    m = x.shape[0] // split
    parts = [lax.dot_general(x[k * m:(k + 1) * m], w, dims, preferred_element_type=f32) for k in range(split)]
    return parts[0] if split == 1 else jnp.concatenate(parts, axis=0)


def _tile(n):
    return slice(n * 128, (n + 1) * 128)


def _kernel(x_hbm, wqkv_hbm, wo_hbm, wg_hbm, wu_hbm, wd_hbm, o_hbm,
            x_sc, xn_sc, xs_sc, ws_sc, hs_sc, ds_sc, q_sc, kv_sc, a_sc, h_sc, h2_sc, o_sc,
            wg_sc, wu_sc, wt_sc, wo_sc, wd_sc, wqkv_raw, wq_sc, wk_sc, wv_sc, wo_raw, tr_sc, sems, osem):
    i = pl.program_id(0)
    z = lax.shift_right_logical(i, 20)
    z16 = pl.multiple_of(z * 16, 16)
    scale = DH ** -0.5 * 1.4426950408889634
    wp_sc = (wq_sc, wk_sc, wv_sc)
    part = functools.partial

    copies = {}

    def mk(name, src, dst):
        copies[name] = pltpu.make_async_copy(src, dst, sems.at[len(copies)])

    def mk_gu(c0, c1):
        mk('g%d' % c0, wg_hbm.at[c0 * FC:c1 * FC, :], wg_sc.at[c0 * FC:c1 * FC, :])
        mk('u%d' % c0, wu_hbm.at[c0 * FC:c1 * FC, :], wu_sc.at[c0 * FC:c1 * FC, :])

    mk('x0', x_hbm.at[0:HT, :], x_sc.at[0:HT, :])
    mk('x1', x_hbm.at[HT:TM0, :], x_sc.at[HT:TM0, :])
    mk_gu(0, 1)
    mk_gu(1, 3)
    mk_gu(3, 7)
    mk('qk', wqkv_hbm.at[:, 0:2 * D], wqkv_raw.at[0:D, 0:2 * D])
    mk_gu(7, 10)
    mk('v', wqkv_hbm.at[:, 2 * D:3 * D], wqkv_raw.at[0:D, 2 * D:3 * D])
    mk_gu(10, NCH)
    mk('wo', wo_hbm, wo_raw)
    mk('gt', wg_hbm.at[FMAIN:F, :], wt_sc.at[0:64, :])
    mk('ut', wu_hbm.at[FMAIN:F, :], wt_sc.at[64:128, :])
    mk('x2', x_hbm.at[TM0:TM0 + TM, :], x_sc.at[TM0:TM0 + TM, :])
    mk('wd', wd_hbm, wd_sc.at[0:F, :])
    mk('x3', x_hbm.at[TM0 + TM:S, :], x_sc.at[TM0 + TM:S, :])

    def wait(*names):
        for n in names:
            copies[n].wait()

    def tok(ref):
        return _upk(ref[pl.ds(z16, 16), 0:128])[0:16]

    def before(ref, val):
        n = ref.shape[0]
        v = val[0:16, 0:128].astype(bf16)
        if ref.dtype == u32:
            ref[pl.ds(n - 16 + z16, 8), 0:128] = pltpu.bitcast(v, u32)
        else:
            ref[pl.ds(n - 16 + z16, 16), 0:128] = v

    def before_q(val):
        q_sc[NT + z, 0:8, :] = val[0:8, 0:128]

    def run(units, pieces=()):
        due, res = {}, {}

        def emit(k):
            for su, srow, fence, thunk, du, *lag in pieces:
                if su + sum(lag) == k:
                    if su >= 0 and fence is not None:
                        fence(res[su][srow:srow + 16])
                    t = thunk()
                    if du is not None:
                        due.setdefault(du, []).append(t())

        emit(-1)
        for k, (ref, thunk) in enumerate(units):
            for t in due.get(k, []):
                before(ref, t)
            res[k] = thunk()
            emit(k)

    def bits(v):
        return pltpu.bitcast(v.astype(f32), u32)

    def gather(slot, lo, hi, t):
        for d in range(DH):
            g = tr_sc[slot, pl.ds(d, H, stride=DH), :]
            rows = slice(d * H // 2, (d + 1) * H // 2)
            lo[rows, _tile(t)] = _pk(pltpu.bitcast(g << 16, f32))
            hi[rows, _tile(t)] = _pk(pltpu.bitcast(g & jnp.uint32(0xFFFF0000), f32))
        return lambda: tok(lo) + tok(hi)

    def perm_qk(t):
        for j in range(NT):
            w = (bits(wqkv_raw[_tile(t), _tile(j)]) >> 16) | bits(wqkv_raw[_tile(t), _tile(NT + j)])
            tr_sc[t % 2, _tile(j), :] = w.T
        return gather(t % 2, wq_sc, wk_sc, t)

    def perm_vo(t):
        for j in range(NT):
            vt = bits(wqkv_raw[_tile(t), _tile(2 * NT + j)]).T
            tr_sc[t % 2, _tile(j), :] = (vt >> 16) | bits(wo_raw[_tile(j), _tile(t)])
        return gather(t % 2, wv_sc, wo_sc, t)

    def wref(tile):
        return wp_sc[tile[1] // NT] if tile[0] == 'p' else (wg_sc if tile[0] == 'g' else wu_sc)

    def wrows(tile, cols, r0=0, nr=128):
        m, n = tile
        if m == 'p':
            return _upk(wref(tile)[(n % NT) * 64 + r0 // 2:(n % NT) * 64 + (r0 + nr) // 2, cols])
        return wref(tile)[n * FC + r0:n * FC + r0 + nr, cols]

    def orows(kt, n, r0=0, nr=128):
        if kt <= NCH:
            return wd_sc[kt * FC + r0:kt * FC + r0 + nr, _tile(n)]
        kt -= NCH + 1
        return _upk(wo_sc[(kt * 128 + r0) // 2:(kt * 128 + r0 + nr) // 2, _tile(n)])

    def before_w(p, val):
        t1, t2 = PAIRS[p]
        before(wref(t1), val)
        if wref(t2) is not wref(t1):
            before(wref(t2), val)

    def wcomb(p, r0, nr):
        t1, t2 = PAIRS[p]
        for t in range(2):
            b11, b21, b12, b22 = [wrows(tl, _tile(c), r0, nr).astype(f32) for tl in (t1, t2) for c in (t, 2 + t)]
            for j, v in enumerate(_rcomb(b11, b12, b21, b22)):
                ws_sc[(p * 5 + j) * 64 + r0 // 2:(p * 5 + j) * 64 + (r0 + nr) // 2, _tile(t)] = _pk(v)
        return lambda: tok(ws_sc)

    def dcomb(kp, r0, nr):
        for q in range(2):
            blk = [orows(k, n, r0, nr).astype(f32) for k in (2 * kp, 2 * kp + 1) for n in (2 * q, 2 * q + 1)]
            for j, v in enumerate(_rcomb(*blk)):
                base = ((q * 5 + j) * KD + kp * 128 + r0) // 2
                ds_sc[base:base + nr // 2, :] = _pk(v)
        return lambda: tok(ds_sc)

    def xcomb(r0):
        blk = lambda h, t: _upk(xn_sc[(h + r0) // 2:(h + r0 + LR) // 2, _tile(t)]).astype(f32)
        for t in range(2):
            for j, v in enumerate(_lcomb(blk(0, t), blk(0, 2 + t), blk(HM, t), blk(HM, 2 + t))):
                xs_sc[r0 // 2:(r0 + LR) // 2, _tile(2 * j + t)] = _pk(v)
        return lambda: tok(xs_sc)

    def hcomb(hm, kp, r0, nr):
        blk = lambda h, c: _upk(h2_sc[(h + r0) // 2:(h + r0 + nr) // 2, _tile(c)]).astype(f32)
        for j, v in enumerate(_lcomb(blk(0, 2 * kp), blk(0, 2 * kp + 1), blk(hm, 2 * kp), blk(hm, 2 * kp + 1))):
            hs_sc[r0 // 2:(r0 + nr) // 2, _tile(j * NKP + kp)] = _pk(v)
        return lambda: tok(hs_sc)

    def acomb(r0):
        blk = lambda h, t: a_sc[h + r0:h + r0 + 16, _tile(t)].astype(f32)
        for kp in range(2):
            for j, v in enumerate(_lcomb(blk(0, 2 * kp), blk(0, 2 * kp + 1), blk(HM, 2 * kp), blk(HM, 2 * kp + 1))):
                hs_sc[r0 // 2:r0 // 2 + 8, _tile(j * NKP + NKH + kp)] = _pk(v)

    def ln_rows(base, r0, n):
        for t, v in enumerate(_ln(x_sc, pl.ds(base + r0, n))):
            xn_sc[r0 // 2:(r0 + n) // 2, _tile(t)] = _pk(v)

    def ln_pieces(base, slots, gap):
        out = []
        for j, r0 in enumerate(range(0, HM, LR)):
            (u1, s1), (u2, s2) = slots[2 * j], slots[2 * j + 1]
            out.append((u1, s1, part(before, x_sc), part(ln_rows, base, r0, LR), None))
            out.append((u2, s2, part(before, x_sc), part(ln_rows, base, HM + r0, LR), None))
            out.append((u2, s2, None, part(xcomb, r0), u2 + gap))
        return out

    def attn(r0, first):
        q = [q_sc[t, r0:r0 + RC, :] for t in range(NT)]
        logits = []
        for w in range(W):
            off = r0 + HALO - w * DIL
            s = q[0] * kv_sc[0, off:off + RC, :]
            for t in range(1, NT):
                s = s + q[t] * kv_sc[t, off:off + RC, :]
            s = s + pltpu.roll(s, 64, 1)
            s = s + pltpu.roll(s, 32, 1)
            if first and w > 0 and r0 < HALO:
                pos = r0 + lax.broadcasted_iota(jnp.int32, (RC, 128), 0)
                s = jnp.where(pos >= w * DIL, s, -1e9)
            logits.append(s)
        m = logits[0]
        for w in range(1, W):
            m = jnp.maximum(m, logits[w])
        p = [jnp.exp2(l - m) for l in logits]
        inv = pl.reciprocal(sum(p[1:], p[0]), approx=True)
        for t in range(NT):
            acc = p[0] * kv_sc[NT + t, r0 + HALO:r0 + HALO + RC, :]
            for w in range(1, W):
                off = r0 + HALO - w * DIL
                acc = acc + p[w] * kv_sc[NT + t, off:off + RC, :]
            a_sc[r0:r0 + RC, _tile(t)] = (acc * inv).astype(bf16)

    def attn_rows(rr, first):
        for r0 in rr:
            attn(r0, first)
            if not first and r0 >= HM and r0 % 16 == 8:
                acomb(r0 - HM - 8)

    def attn_pieces(slots, first):
        if first:
            rows = list(range(0, TM0, RC))
        else:
            rows = [h + r + e for r in range(0, HM, 16) for h in (0, HM) for e in (0, 8)]
        n, out = len(rows), []
        for j, (u, srow) in enumerate(slots):
            rr = rows[-(-j * n // len(slots)):-(-(j + 1) * n // len(slots))]
            if rr:
                out.append((u, srow, before_q, part(attn_rows, rr, first), None))
        return out

    class Block:
        def __init__(self, tm):
            self.tm, self.g = tm, {}
            self.xn = _upk(xn_sc[0:tm // 2, :])
            self.xs = _upk(xs_sc[...]) if tm == TM else None

        def put_h(self, c, h):
            hp = _pk(h)
            h_sc[0:self.tm // 2, _tile(c)] = hp
            h2_sc[0:self.tm // 2, _tile(c)] = hp

        def finish(self, tile, r):
            m, n = tile
            if m == 'g':
                self.g[n] = r
            elif m == 'u':
                self.put_h(n, _gelu(self.g[n]) * r)
            elif n < NT:
                q_sc[n, 0:self.tm, :] = r * scale
            else:
                kv_sc[n - NT, HALO:HALO + self.tm, :] = r

        def plain(self, tile, split):
            r = _dot(self.xn, wrows(tile, slice(0, D)), NT_DIMS, split)
            self.finish(tile, r)
            return r

        def tail(self):
            gu = _dot(self.xn, wt_sc[0:128, :], NT_DIMS)
            h = _gelu(gu) * pltpu.roll(gu, 64, 1)
            lane = lax.broadcasted_iota(jnp.int32, gu.shape, 1)
            self.put_h(NCH, jnp.where(lane < 64, h, 0.0))
            return gu

        def P(self, ns):
            return [(wref(('p', n)), part(self.plain, ('p', n), 1)) for n in ns]

        def GU(self, cs, split=1):
            return [(wref((m, c)), part(self.plain, (m, c), split)) for c in cs for m in 'gu']

        def T(self):
            return [(wt_sc, self.tail)]

        def S(self, p):
            t1, t2 = PAIRS[p]
            xn, k5 = self.xn, slice(2 * KS, D)
            xs = lambda j: self.xs[:, j * KS:(j + 1) * KS]
            ws = lambda j: _upk(ws_sc[(p * 5 + j) * 64:(p * 5 + j + 1) * 64, :])
            cat = lambda *v: jnp.concatenate(v, axis=1)
            ops = {
                1: (ws_sc, lambda: (xs(0), ws(0))),
                2: (wref(t1), lambda: (xs(1), wrows(t1, slice(0, KS)))),
                3: (ws_sc, lambda: (xn[0:HM, 0:KS], ws(1))),
                4: (ws_sc, lambda: (xn[HM:TM, KS:2 * KS], ws(2))),
                5: (wref(t2), lambda: (xs(2), wrows(t2, slice(KS, 2 * KS)))),
                6: (ws_sc, lambda: (cat(xs(3), xn[HM:TM, k5]), cat(ws(3), wrows(t2, k5)))),
                7: (ws_sc, lambda: (cat(xs(4), xn[0:HM, k5]), cat(ws(4), wrows(t1, k5)))),
                8: (wref(t1), lambda: (xn[HM:TM, k5], wrows(t1, k5))),
                9: (wref(t2), lambda: (xn[0:HM, k5], wrows(t2, k5))),
            }
            m = {}

            def prod(k):
                m[k] = _dot(*ops[k][1](), NT_DIMS)
                if len(m) == 9:
                    self.finish(t1, jnp.concatenate([(m[4] - m[5]) + (m[1] + m[7]), (m[8] + m[4]) + m[2]], axis=0))
                    self.finish(t2, jnp.concatenate([(m[9] + m[5]) + m[3], (m[1] + (m[3] - m[2])) + m[6]], axis=0))
                return m[k]

            return [(ops[k][0], part(prod, k)) for k in (4, 5, 7, 8, 1, 2, 3, 9, 6)]

    def out_ops(hm, q, nkp, a):
        hs = lambda j: _upk(hs_sc[0:hm // 2, j * KD:j * KD + nkp * 128])
        ds = lambda j: _upk(ds_sc[(q * 5 + j) * KD // 2:((q * 5 + j) * KD + nkp * 128) // 2, :])
        hq = lambda half, par: jnp.concatenate(
            [_upk(h_sc[half * hm // 2:(half + 1) * hm // 2, _tile(k)]) if k <= NCH else
             a[half * hm:(half + 1) * hm, _tile(k - NCH - 1)] for k in range(par, 2 * nkp, 2)], axis=1)
        dq = lambda par: jnp.concatenate([orows(k, 2 * q + par) for k in range(par, 2 * nkp, 2)], axis=0)
        return {1: lambda: (hs(0), ds(0)), 2: lambda: (hs(1), dq(0)), 3: lambda: (hq(0, 0), ds(1)),
                4: lambda: (hq(1, 1), ds(2)), 5: lambda: (hs(2), dq(1)), 6: lambda: (hs(3), ds(3)),
                7: lambda: (hs(4), ds(4)), 8: lambda: (a[:, _tile(NT - 1)], orows(2 * NKP, 2 * q)),
                9: lambda: (a[:, _tile(NT - 1)], orows(2 * NKP, 2 * q + 1))}

    def emit_out(row0, n, y):
        rows = pl.ds(row0, y.shape[0])
        o_sc[rows, _tile(n)] = (x_sc[rows, _tile(n)].astype(f32) + y).astype(bf16)
        pltpu.make_async_copy(o_sc.at[rows, _tile(n)], o_hbm.at[rows, _tile(n)], osem).start()

    def halo(tm):
        kv_sc[:, 0:HALO, :] = kv_sc[:, tm:tm + HALO, :]

    @pl.when(i == 0)
    def _():
        for cp in copies.values():
            cp.start()
        kv_sc[:, 0:HALO, :] = jnp.zeros((2 * NT, HALO, 128), f32)
        wd_sc[F:FP, :] = jnp.zeros((FP - F, D), bf16)
        for ref in (xs_sc, ws_sc, hs_sc, ds_sc):
            ref[0:16, 0:128] = jnp.zeros((16, 128), u32)
        wait('x0')
        for r0 in range(0, HT, 64):
            ln_rows(0, r0, 64)
        wait('x1')
        for r0 in range(HT, TM0, 64):
            ln_rows(0, r0, 64)
        wait('g0', 'u0')
        b = Block(TM0)

        def tiny(todo, u0, last, off=0):
            return [(u0 + j // 8, (j % 8) * 64 + off, f, th, min(u0 + j // 8 + 3, last) if j % 8 == 7 else None, 1)
                    for j, (f, th) in enumerate(todo)]

        wc = lambda ps: [(part(before_w, p), part(wcomb, p, r0, 16)) for p in ps for r0 in range(0, 128, 16)]
        hc = lambda kps: [(part(before, h2_sc), part(hcomb, HT, kp, r0, 32)) for kp in kps for r0 in range(0, HT, 32)]
        dc = lambda kps: [(part(before, wd_sc if kp < NKH else wo_sc), part(dcomb, kp, r0, 16))
                          for kp in kps for r0 in range(0, 128, 16)]

        run(b.GU([0], 2))
        wait('g1', 'u1')
        run(b.GU([1, 2]), tiny(wc([7]), 0, 3))
        wait('g3', 'u3')
        run(b.GU([3, 4, 5, 6]), tiny(wc([8, 9, 10, 11, 12]), 0, 7))
        wait('qk', 'g7', 'u7')
        run(b.GU([7, 8, 9]) + b.P(range(10)),
            [(max(t - 2, -1), 0, part(before, wqkv_raw), part(perm_qk, t), t + 2) for t in range(NT)]
            + tiny(wc([13, 14, 15, 16, 0, 1, 2, 3, 6]), 4, 15) + tiny(hc(range(5)), 6, 15, 32))
        wait('v', 'g10', 'u10', 'wo', 'gt', 'ut', 'x2', 'wd')

        acc = {0: {}, 1: {}}

        def down_last(half):
            ks = slice(half * FP // 2, (half + 1) * FP // 2)
            y = _dot(_upk(h_sc[0:TM0 // 2, ks]), wd_sc[ks, _tile(NT - 1)], NN_DIMS)
            acc['y', NT - 1] = y if half == 0 else acc['y', NT - 1] + y
            return y

        def down(q, k):
            m = acc[q]
            m[k] = _dot(*out_ops(HT, q, NKH, None)[k](), NN_DIMS)
            if len(m) == 7:
                acc['y', 2 * q], acc['y', 2 * q + 1] = _ocomb(m)
            return m[k]

        def oproj(n):
            if n == 0:
                halo(TM0)
                acc['a'] = a_sc[0:TM0, :]
            y = _dot(acc['a'], _upk(wo_sc[0:D // 2, _tile(n)]), NN_DIMS, 4 if n == NT - 1 else 1)
            emit_out(0, n, acc['y', n] + y)
            return y

        units = (b.GU([10, 11, 12]) + b.T() + b.P(range(10, 15))
                 + [(wd_sc, part(down_last, half)) for half in range(2)]
                 + [(wd_sc if k in (2, 5) else ds_sc, part(down, q, k))
                    for q in range(2) for k in (4, 5, 1, 7, 2, 3, 6)]
                 + [(wo_sc, part(oproj, n)) for n in range(NT)])
        when = [(-1, 2), (-1, 3), (1, 4), (2, 5), (3, 6)]
        pieces = [(su, 0, part(before, wqkv_raw), part(perm_vo, t), du) for t, (su, du) in enumerate(when)]
        pieces += tiny(dc(range(NKH)), 4, 14)
        pieces += tiny(wc([17, 18]), 5, 32, 32)
        pieces += tiny(dc([NKH, NKH + 1]), 7, 32, 32)
        pieces += tiny(hc([5, 6]), 9, 14, 32)
        pieces += tiny(wc([4, 5]), 11, 32, 32)
        pieces += ln_pieces(TM0 + z16, [(u, r) for u in (26, 27) for r in range(0, HT, 64)]
                            + [(u, r) for u in (28, 29) for r in range(0, TM0, 64)], 3)
        pieces += attn_pieces([(u, r) for u in range(11, 14) for r in range(0, TM0, 128)]
                              + [(u, r) for u in range(14, 25) for r in range(0, HT, 128)], True)
        run(units, pieces)
        wait('x3')

    @pl.when(i > 0)
    def _():
        row0 = pl.multiple_of(TM0 + (i - 1) * TM, 16)
        nxt = pl.multiple_of(jnp.minimum(row0 + TM, S - TM), 16)
        b = Block(TM)
        units = [u for p in range(7) for u in b.S(p)] + b.P([14])
        nq = len(units)
        units += [u for p in range(7, len(PAIRS)) for u in b.S(p)] + b.GU([12]) + b.T()
        nf = len(units)
        st = {0: {}, 1: {}}

        def last_tile(half):
            if half == 0:
                halo(TM)
                st['a'] = a_sc[0:TM, :]
                kts = list(range(NCH + 1, 2 * NKP + 1)) + list(range(4))
            else:
                kts = list(range(4, NCH + 1))
            lhs = jnp.concatenate([_upk(h_sc[0:TM // 2, _tile(k)]) if k <= NCH else st['a'][:, _tile(k - NCH - 1)]
                                   for k in kts], axis=1)
            y = _dot(lhs, jnp.concatenate([orows(k, NT - 1) for k in kts], axis=0), NN_DIMS)
            if half == 0:
                st['y'] = y
            else:
                emit_out(row0, NT - 1, st['y'] + y)
            return y

        def prod(q, k):
            m = st[q]
            m[k] = _dot(*out_ops(HM, q, NKP, st['a'])[k](), NN_DIMS)
            if len(m) == 9:
                c1, c2 = _ocomb(m)
                c1, c2 = c1 + m[8], c2 + m[9]
                emit_out(row0, 2 * q, c1)
                emit_out(row0, 2 * q + 1, c2[0:HM])
                emit_out(row0 + HM, 2 * q + 1, c2[HM:TM])
            return m[k]

        units += [(wd_sc, part(last_tile, 0)), (wd_sc, part(last_tile, 1))]
        units += [(ds_sc, part(prod, q, k)) for q, k in
                  [(0, 4), (0, 3), (1, 4), (1, 3)] + [(q, k) for q in range(2) for k in (8, 9, 2, 5, 1, 7, 6)]]
        pieces = ln_pieces(nxt, [(2 * j, 0) for j in range(TM // LR)], 8)
        pieces += attn_pieces([(u, 0) for u in range(nq - 1, nf - 2)], False)
        slots = ([(u, r) for u in range(nf, nf + 2) for r in range(0, TM, 32)]
                 + [(u, r) for u in range(nf + 2, nf + 5) for r in range(0, HM, 32)])
        todo = [(kp, r0) for kp in range(NKH) for r0 in range(0, HM, 32)]
        pieces += [(u, r, part(before, h2_sc), part(hcomb, HM, kp, r0, 32), None) for (u, r), (kp, r0) in zip(slots, todo)]
        run(units, pieces)

    @pl.when(i == NB - 1)
    def _():
        pltpu.make_async_copy(o_sc, o_hbm, osem).wait()


@jax.jit
def pallas_parallel_sum__sliding_local_dilated__geglu_ffn__prompt_kernel(
    A_x: jax.Array,
    A_wqkv: jax.Array,
    A_wo: jax.Array,
    B_x: jax.Array,
    B_w_gate: jax.Array,
    B_w_up: jax.Array,
    B_w_down: jax.Array,
):
    assert A_x.shape == (1, S, D) and B_w_gate.shape == (D, F)
    hbm = pl.BlockSpec(memory_space=pl.ANY)
    out = pl.pallas_call(
        _kernel,
        grid=(NB,),
        in_specs=[hbm] * 6,
        out_specs=hbm,
        out_shape=jax.ShapeDtypeStruct((S, D), A_x.dtype),
        scratch_shapes=[
            pltpu.VMEM((S + 16, D), bf16),
            pltpu.VMEM((TMX // 2, D), u32),
            pltpu.VMEM((HM // 2, 5 * KS), u32),
            pltpu.VMEM((len(PAIRS) * 5 * 64 + 16, KS), u32),
            pltpu.VMEM((TMX // 4, 5 * KD), u32),
            pltpu.VMEM((10 * KD // 2 + 16, 128), u32),
            pltpu.VMEM((NT + 1, TMX, 128), f32),
            pltpu.VMEM((2 * NT, TMX + HALO, 128), f32),
            pltpu.VMEM((TMX, D), bf16),
            pltpu.VMEM((TMX // 2, FP), u32),
            pltpu.VMEM((TMX // 2 + 16, FP), u32),
            pltpu.VMEM((S, D), bf16),
            pltpu.VMEM((FMAIN + 16, D), bf16),
            pltpu.VMEM((FMAIN + 16, D), bf16),
            pltpu.VMEM((128 + 16, D), bf16),
            pltpu.VMEM((D // 2 + 16, D), u32),
            pltpu.VMEM((FP + 16, D), bf16),
            pltpu.VMEM((D + 16, 3 * D), bf16),
            pltpu.VMEM((D // 2 + 16, D), u32),
            pltpu.VMEM((D // 2 + 16, D), u32),
            pltpu.VMEM((D // 2 + 16, D), u32),
            pltpu.VMEM((D, D), bf16),
            pltpu.VMEM((2, D + 32, 128), u32),
            pltpu.SemaphoreType.DMA((20,)),
            pltpu.SemaphoreType.DMA(()),
        ],
        compiler_params=pltpu.CompilerParams(
            dimension_semantics=("arbitrary",),
            vmem_limit_bytes=100 * 1024 * 1024,
            disable_semaphore_checks=True,
            disable_bounds_checks=True,
        ),
    )(A_x.reshape(S, D), A_wqkv, A_wo, B_w_gate.T, B_w_up.T, B_w_down)
    return out.reshape(1, S, D)
```

```python
import functools

import jax
import jax.numpy as jnp
from jax import lax
import jax.experimental.pallas as pl
import jax.experimental.pallas.tpu as pltpu

S, D, F = 2048, 640, 1728
H, DH, W, DIL = 32, 20, 8, 2
HALO = 16
TM0 = 512
TM = 384
NB = 1 + (S - TM0) // TM
TMX = max(TM, TM0)
HT, HM = TM0 // 2, TM // 2
NT = D // 128
FC = 128
NCH = F // FC
FP = (NCH + 1) * FC
RC = 8
LR = 16
KS = 256
NKH = (NCH + 1) // 2
NKP = NKH + 2
KD = NKP * 128
PAIRS = ([(('p', a), ('p', a + 1)) for a in (0, 2, 5, 7, 10, 12)] + [(('p', 4), ('p', 9))]
         + [((m, c), (m, c + 1)) for c in range(0, 12, 2) for m in 'gu'] + [(('t', 0), ('t', 1))])
NT_DIMS = (((1,), (1,)), ((), ()))
NN_DIMS = (((1,), (0,)), ((), ()))
f32, bf16, u32 = jnp.float32, jnp.bfloat16, jnp.uint32


def _pk(v):
    return pltpu.bitcast(v.astype(bf16), u32)


def _upk(v):
    return pltpu.bitcast(v, bf16)


def _gelu2(g):
    c = 0.7978845608028654
    return g * (1.0 + jnp.tanh(g * (c + (c * 0.044715) * (g * g))))


def _ln(ref, rows):
    x = [ref[rows, t * 128:(t + 1) * 128].astype(f32) for t in range(NT)]
    mu = jnp.sum(sum(x[1:], x[0]), axis=-1, keepdims=True) * (1.0 / D)
    mb = mu.astype(bf16).astype(f32)
    xc = [v - mb for v in x]
    sq = [v * v for v in xc]
    var = jnp.sum(sum(sq[1:], sq[0]), axis=-1, keepdims=True) * (1.0 / D) - (mu - mb) * (mu - mb)
    r = lax.rsqrt(jnp.maximum(var, 0.0) + 1e-5)
    return [v * r for v in xc]


def _lcomb(a11, a12, a21, a22):
    return a11 + a22, a21 + a22, a11 + a12, a21 - a11, a12 - a22


def _rcomb(b11, b12, b21, b22):
    return b11 + b22, b12 - b22, b21 - b11, b11 + b12, b21 + b22


def _ocomb(m):
    return (jnp.concatenate([(m[4] - m[5]) + (m[1] + m[7]), m[4] + m[2]], axis=0),
            jnp.concatenate([m[5] + m[3], (m[1] + (m[3] - m[2])) + m[6]], axis=0))


def _dot(x, w, dims, split=1):
    m = x.shape[0] // split
    parts = [lax.dot_general(x[k * m:(k + 1) * m], w, dims, preferred_element_type=f32) for k in range(split)]
    return parts[0] if split == 1 else jnp.concatenate(parts, axis=0)


def _tile(n):
    return slice(n * 128, (n + 1) * 128)


def _kernel(x_hbm, wqkv_hbm, wo_hbm, wg_hbm, wu_hbm, wd_hbm, o_hbm,
            x_sc, xn_sc, xs_sc, ws_sc, hs_sc, ds_sc, q_sc, kv_sc, a_sc, h_sc, h2_sc, o_sc,
            wg_sc, wu_sc, wt_sc, wo_sc, wd_sc, wqkv_raw, wq_sc, wk_sc, wv_sc, wo_raw, tr_sc, sems, osem):
    i = pl.program_id(0)
    z = lax.shift_right_logical(i, 20)
    z16 = pl.multiple_of(z * 16, 16)
    scale = DH ** -0.5 * 1.4426950408889634
    wp_sc = (wq_sc, wk_sc, wv_sc)
    part = functools.partial

    copies = {}

    def mk(name, src, dst):
        copies[name] = pltpu.make_async_copy(src, dst, sems.at[len(copies)])

    def mk_gu(c0, c1):
        mk('g%d' % c0, wg_hbm.at[c0 * FC:c1 * FC, :], wg_sc.at[c0 * FC:c1 * FC, :])
        mk('u%d' % c0, wu_hbm.at[c0 * FC:c1 * FC, :], wu_sc.at[c0 * FC:c1 * FC, :])

    mk('x0', x_hbm.at[0:HT, :], x_sc.at[0:HT, :])
    mk('x1', x_hbm.at[HT:TM0, :], x_sc.at[HT:TM0, :])
    mk_gu(0, 1)
    mk_gu(1, 3)
    mk_gu(3, 7)
    mk('qk', wqkv_hbm.at[:, 0:2 * D], wqkv_raw.at[0:D, 0:2 * D])
    mk_gu(7, 10)
    mk('v', wqkv_hbm.at[:, 2 * D:3 * D], wqkv_raw.at[0:D, 2 * D:3 * D])
    mk_gu(10, 12)
    mk('wo', wo_hbm, wo_raw)
    for j in range(3):
        r0 = 12 * FC + j * 64
        mk('gt%d' % j, wg_hbm.at[r0:r0 + 64, :], wt_sc.at[j * 128:j * 128 + 64, :])
        mk('ut%d' % j, wu_hbm.at[r0:r0 + 64, :], wt_sc.at[j * 128 + 64:(j + 1) * 128, :])
    mk('x2', x_hbm.at[TM0:TM0 + TM, :], x_sc.at[TM0:TM0 + TM, :])
    mk('wd', wd_hbm, wd_sc.at[0:F, :])
    mk('x3', x_hbm.at[TM0 + TM:S, :], x_sc.at[TM0 + TM:S, :])

    def wait(*names):
        for n in names:
            copies[n].wait()

    def tok(ref):
        return _upk(ref[pl.ds(z16, 16), 0:128])[0:16]

    def before(ref, val):
        n = ref.shape[0]
        v = val[0:16, 0:128].astype(bf16)
        if ref.dtype == u32:
            ref[pl.ds(n - 16 + z16, 8), 0:128] = pltpu.bitcast(v, u32)
        else:
            ref[pl.ds(n - 16 + z16, 16), 0:128] = v

    def before_q(val):
        q_sc[NT + z, 0:8, :] = val[0:8, 0:128]

    def run(units, pieces=()):
        due, res = {}, {}

        def emit(k):
            for su, srow, fence, thunk, du, *lag in pieces:
                if su + sum(lag) == k:
                    if su >= 0 and fence is not None:
                        fence(res[su][srow:srow + 16])
                    t = thunk()
                    if du is not None:
                        due.setdefault(du, []).append(t())

        emit(-1)
        for k, (ref, thunk) in enumerate(units):
            for t in due.get(k, []):
                before(ref, t)
            res[k] = thunk()
            emit(k)

    def bits(v):
        return pltpu.bitcast(v.astype(f32), u32)

    def gather(slot, lo, hi, t):
        for d in range(DH):
            g = tr_sc[slot, pl.ds(d, H, stride=DH), :]
            rows = slice(d * H // 2, (d + 1) * H // 2)
            lo[rows, _tile(t)] = _pk(pltpu.bitcast(g << 16, f32))
            hi[rows, _tile(t)] = _pk(pltpu.bitcast(g & jnp.uint32(0xFFFF0000), f32))
        return lambda: tok(lo) + tok(hi)

    def perm_qk(t):
        for j in range(NT):
            w = (bits(wqkv_raw[_tile(t), _tile(j)]) >> 16) | bits(wqkv_raw[_tile(t), _tile(NT + j)])
            tr_sc[t % 2, _tile(j), :] = w.T
        return gather(t % 2, wq_sc, wk_sc, t)

    def perm_vo(t):
        for j in range(NT):
            vt = bits(wqkv_raw[_tile(t), _tile(2 * NT + j)]).T
            tr_sc[t % 2, _tile(j), :] = (vt >> 16) | bits(wo_raw[_tile(j), _tile(t)])
        return gather(t % 2, wv_sc, wo_sc, t)

    def wref(tile):
        return wp_sc[tile[1] // NT] if tile[0] == 'p' else {'g': wg_sc, 'u': wu_sc, 't': wt_sc}[tile[0]]

    def wrows(tile, cols, r0=0, nr=128):
        m, n = tile
        if m == 'p':
            return _upk(wref(tile)[(n % NT) * 64 + r0 // 2:(n % NT) * 64 + (r0 + nr) // 2, cols])
        return wref(tile)[n * FC + r0:n * FC + r0 + nr, cols]

    def orows(kt, n, r0=0, nr=128):
        if kt <= NCH:
            return wd_sc[kt * FC + r0:kt * FC + r0 + nr, _tile(n)]
        kt -= NCH + 1
        return _upk(wo_sc[(kt * 128 + r0) // 2:(kt * 128 + r0 + nr) // 2, _tile(n)])

    def before_w(p, val):
        t1, t2 = PAIRS[p]
        before(wref(t1), val)
        if wref(t2) is not wref(t1):
            before(wref(t2), val)

    def wcomb(p, r0, nr):
        t1, t2 = PAIRS[p]
        for t in range(2):
            b11, b21, b12, b22 = [wrows(tl, _tile(c), r0, nr).astype(f32) for tl in (t1, t2) for c in (t, 2 + t)]
            for j, v in enumerate(_rcomb(b11, b12, b21, b22)):
                ws_sc[(p * 5 + j) * 64 + r0 // 2:(p * 5 + j) * 64 + (r0 + nr) // 2, _tile(t)] = _pk(v)
        return lambda: tok(ws_sc)

    def dcomb(kp, r0, nr):
        for q in range(2):
            blk = [orows(k, n, r0, nr).astype(f32) for k in (2 * kp, 2 * kp + 1) for n in (2 * q, 2 * q + 1)]
            for j, v in enumerate(_rcomb(*blk)):
                base = (j * KD + kp * 128 + r0) // 2
                ds_sc[base:base + nr // 2, _tile(q)] = _pk(v)
        return lambda: tok(ds_sc)

    def xcomb(r0):
        blk = lambda h, t: _upk(xn_sc[(h + r0) // 2:(h + r0 + LR) // 2, _tile(t)]).astype(f32)
        for t in range(2):
            for j, v in enumerate(_lcomb(blk(0, t), blk(0, 2 + t), blk(HM, t), blk(HM, 2 + t))):
                xs_sc[r0 // 2:(r0 + LR) // 2, _tile(2 * j + t)] = _pk(v)
        return lambda: tok(xs_sc)

    def hcomb(hm, kp, r0, nr):
        blk = lambda h, c: _upk(h2_sc[(h + r0) // 2:(h + r0 + nr) // 2, _tile(c)]).astype(f32)
        for j, v in enumerate(_lcomb(blk(0, 2 * kp), blk(0, 2 * kp + 1), blk(hm, 2 * kp), blk(hm, 2 * kp + 1))):
            hs_sc[r0 // 2:(r0 + nr) // 2, _tile(j * NKP + kp)] = _pk(v)
        return lambda: tok(hs_sc)

    def acomb(r0):
        blk = lambda h, t: a_sc[h + r0:h + r0 + 16, _tile(t)].astype(f32)
        for kp in range(2):
            for j, v in enumerate(_lcomb(blk(0, 2 * kp), blk(0, 2 * kp + 1), blk(HM, 2 * kp), blk(HM, 2 * kp + 1))):
                hs_sc[r0 // 2:r0 // 2 + 8, _tile(j * NKP + NKH + kp)] = _pk(v)

    def ln_rows(base, r0, n):
        for t, v in enumerate(_ln(x_sc, pl.ds(base + r0, n))):
            xn_sc[r0 // 2:(r0 + n) // 2, _tile(t)] = _pk(v)

    def ln_pieces(base, slots, gap):
        out = []
        for j, r0 in enumerate(range(0, HM, LR)):
            (u1, s1), (u2, s2) = slots[2 * j], slots[2 * j + 1]
            out.append((u1, s1, part(before, x_sc), part(ln_rows, base, r0, LR), None))
            out.append((u2, s2, part(before, x_sc), part(ln_rows, base, HM + r0, LR), None))
            out.append((u2, s2, None, part(xcomb, r0), u2 + gap))
        return out

    def attn(r0, first):
        q = [q_sc[t, r0:r0 + RC, :] for t in range(NT)]
        logits = []
        for w in range(W):
            off = r0 + HALO - w * DIL
            s = q[0] * kv_sc[0, off:off + RC, :]
            for t in range(1, NT):
                s = s + q[t] * kv_sc[t, off:off + RC, :]
            s = s + pltpu.roll(s, 64, 1)
            s = s + pltpu.roll(s, 32, 1)
            if first and w > 0 and r0 < HALO:
                pos = r0 + lax.broadcasted_iota(jnp.int32, (RC, 128), 0)
                s = jnp.where(pos >= w * DIL, s, -1e9)
            logits.append(s)
        m = logits[0]
        for w in range(1, W):
            m = jnp.maximum(m, logits[w])
        p = [jnp.exp2(l - m) for l in logits]
        inv = 2.0 * pl.reciprocal(sum(p[1:], p[0]), approx=True)
        for t in range(NT):
            acc = p[0] * kv_sc[NT + t, r0 + HALO:r0 + HALO + RC, :]
            for w in range(1, W):
                off = r0 + HALO - w * DIL
                acc = acc + p[w] * kv_sc[NT + t, off:off + RC, :]
            a_sc[r0:r0 + RC, _tile(t)] = (acc * inv).astype(bf16)

    def attn_rows(rr, first):
        for r0 in rr:
            attn(r0, first)
            if not first and r0 >= HM and r0 % 16 == 8:
                acomb(r0 - HM - 8)

    def attn_pieces(slots, first):
        if first:
            rows = list(range(0, TM0, RC))
        else:
            rows = [h + r + e for r in range(0, HM, 16) for h in (0, HM) for e in (0, 8)]
        n, out = len(rows), []
        for j, (u, srow) in enumerate(slots):
            rr = rows[-(-j * n // len(slots)):-(-(j + 1) * n // len(slots))]
            if rr:
                out.append((u, srow, before_q, part(attn_rows, rr, first), None))
        return out

    class Block:
        def __init__(self, tm):
            self.tm, self.g = tm, {}
            self.xn = _upk(xn_sc[0:tm // 2, :])
            self.xs = _upk(xs_sc[...]) if tm == TM else None

        def put_h(self, c, h):
            hp = _pk(h)
            h_sc[0:self.tm // 2, _tile(c)] = hp
            h2_sc[0:self.tm // 2, _tile(c)] = hp

        def finish(self, tile, r):
            m, n = tile
            if m == 'g':
                self.g[n] = r
            elif m == 'u':
                self.put_h(n, _gelu2(self.g[n]) * r)
            elif m == 't':
                low = lax.broadcasted_iota(jnp.int32, r.shape, 1) < 64
                if n == 0:
                    self.g['t'] = r
                elif n == 1:
                    x_ = self.g['t']
                    sw = pltpu.roll(jnp.where(low, r, x_), 64, 1)
                    self.put_h(NCH - 1, _gelu2(jnp.where(low, x_, sw)) * jnp.where(low, sw, r))
                else:
                    self.put_h(NCH, jnp.where(low, _gelu2(r) * pltpu.roll(r, 64, 1), 0.0))
            elif n < NT:
                q_sc[n, 0:self.tm, :] = r * scale
            else:
                kv_sc[n - NT, HALO:HALO + self.tm, :] = r

        def plain(self, tile, split):
            r = _dot(self.xn, wrows(tile, slice(0, D)), NT_DIMS, split)
            self.finish(tile, r)
            return r

        def P(self, ns):
            return [(wref(('p', n)), part(self.plain, ('p', n), 1)) for n in ns]

        def GU(self, cs, split=1):
            return [(wref((m, c)), part(self.plain, (m, c), split)) for c in cs for m in 'gu']

        def T(self, ns):
            return [(wt_sc, part(self.plain, ('t', n), 1)) for n in ns]

        def gu12(self, m):
            o = 0 if m == 'g' else 64
            w = jnp.concatenate([wt_sc[o:o + 64, :], wt_sc[128 + o:192 + o, :]], axis=0)
            r = _dot(self.xn, w, NT_DIMS)
            self.finish((m, 12), r)
            return r

        def S(self, p):
            t1, t2 = PAIRS[p]
            xn, k5 = self.xn, slice(2 * KS, D)
            xs = lambda j: self.xs[:, j * KS:(j + 1) * KS]
            ws = lambda j: _upk(ws_sc[(p * 5 + j) * 64:(p * 5 + j + 1) * 64, :])
            cat = lambda *v: jnp.concatenate(v, axis=1)
            ops = {
                1: (ws_sc, lambda: (xs(0), ws(0))),
                2: (wref(t1), lambda: (xs(1), wrows(t1, slice(0, KS)))),
                3: (ws_sc, lambda: (xn[0:HM, 0:KS], ws(1))),
                4: (ws_sc, lambda: (xn[HM:TM, KS:2 * KS], ws(2))),
                5: (wref(t2), lambda: (xs(2), wrows(t2, slice(KS, 2 * KS)))),
                6: (ws_sc, lambda: (cat(xs(3), xn[HM:TM, k5]), cat(ws(3), wrows(t2, k5)))),
                7: (ws_sc, lambda: (cat(xs(4), xn[0:HM, k5]), cat(ws(4), wrows(t1, k5)))),
                8: (wref(t1), lambda: (xn[HM:TM, k5], wrows(t1, k5))),
                9: (wref(t2), lambda: (xn[0:HM, k5], wrows(t2, k5))),
            }
            m = {}

            def prod(k):
                m[k] = _dot(*ops[k][1](), NT_DIMS)
                if len(m) == 9:
                    self.finish(t1, jnp.concatenate([(m[4] - m[5]) + (m[1] + m[7]), (m[8] + m[4]) + m[2]], axis=0))
                    self.finish(t2, jnp.concatenate([(m[9] + m[5]) + m[3], (m[1] + (m[3] - m[2])) + m[6]], axis=0))
                return m[k]

            return [(ops[k][0], part(prod, k)) for k in (4, 5, 7, 8, 1, 2, 3, 9, 6)]

    def out_ops(hm, q, nkp, a):
        hs = lambda j: _upk(hs_sc[0:hm // 2, j * KD:j * KD + nkp * 128])
        ds = lambda j: _upk(ds_sc[j * KD // 2:(j * KD + nkp * 128) // 2, _tile(q)])
        hq = lambda half, par: jnp.concatenate(
            [_upk(h_sc[half * hm // 2:(half + 1) * hm // 2, _tile(k)]) if k <= NCH else
             a[half * hm:(half + 1) * hm, _tile(k - NCH - 1)] for k in range(par, 2 * nkp, 2)], axis=1)
        dq = lambda par: jnp.concatenate([orows(k, 2 * q + par) for k in range(par, 2 * nkp, 2)], axis=0)
        return {1: lambda: (hs(0), ds(0)), 2: lambda: (hs(1), dq(0)), 3: lambda: (hq(0, 0), ds(1)),
                4: lambda: (hq(1, 1), ds(2)), 5: lambda: (hs(2), dq(1)), 6: lambda: (hs(3), ds(3)),
                7: lambda: (hs(4), ds(4)), 8: lambda: (a[:, _tile(NT - 1)], orows(2 * NKP, 2 * q)),
                9: lambda: (a[:, _tile(NT - 1)], orows(2 * NKP, 2 * q + 1))}

    def emit_out(row0, n, y):
        rows = pl.ds(row0, y.shape[0])
        o_sc[rows, _tile(n)] = (x_sc[rows, _tile(n)].astype(f32) + 0.5 * y).astype(bf16)
        pltpu.make_async_copy(o_sc.at[rows, _tile(n)], o_hbm.at[rows, _tile(n)], osem).start()

    def halo(tm):
        kv_sc[:, 0:HALO, :] = kv_sc[:, tm:tm + HALO, :]

    @pl.when(i == 0)
    def _():
        for cp in copies.values():
            cp.start()
        kv_sc[:, 0:HALO, :] = jnp.zeros((2 * NT, HALO, 128), f32)
        wd_sc[F:FP, :] = jnp.zeros((FP - F, D), bf16)
        for ref in (xs_sc, ws_sc, hs_sc, ds_sc):
            ref[0:16, 0:128] = jnp.zeros((16, 128), u32)
        wait('x0')
        for r0 in range(0, HT, 64):
            ln_rows(0, r0, 64)
        wait('x1')
        for r0 in range(HT, TM0, 64):
            ln_rows(0, r0, 64)
        wait('g0', 'u0')
        b = Block(TM0)

        def tiny(todo, u0, last, off=0):
            return [(u0 + j // 8, (j % 8) * 64 + off, f, th, min(u0 + j // 8 + 3, last) if j % 8 == 7 else None, 1)
                    for j, (f, th) in enumerate(todo)]

        wc = lambda ps: [(part(before_w, p), part(wcomb, p, r0, 16)) for p in ps for r0 in range(0, 128, 16)]
        hc = lambda kps: [(part(before, h2_sc), part(hcomb, HT, kp, r0, 32)) for kp in kps for r0 in range(0, HT, 32)]
        dc = lambda kps: [(part(before, wd_sc if kp < NKH else wo_sc), part(dcomb, kp, r0, 16))
                          for kp in kps for r0 in range(0, 128, 16)]

        run(b.GU([0], 2))
        wait('g1', 'u1')
        run(b.GU([1, 2]))
        wait('g3', 'u3')
        run(b.GU([3, 4, 5, 6]), tiny(wc([8, 7, 10, 9, 12]), 0, 7))
        wait('qk', 'g7', 'u7')
        run(b.GU([7, 8, 9]) + b.P(range(10)),
            [(max(t - 2, -1), 0, part(before, wqkv_raw), part(perm_qk, t), t + 2) for t in range(NT)]
            + tiny(wc([13, 14, 2, 3, 15, 16, 6, 0, 1]), 4, 15) + tiny(hc(range(5)) + wc([11]), 6, 15, 32))
        wait('v', 'g10', 'u10', 'wo', 'gt0', 'ut0', 'gt1', 'ut1', 'gt2', 'ut2', 'x2', 'wd')

        acc = {0: {}, 1: {}}

        def down_last(half):
            ks = slice(half * FP // 2, (half + 1) * FP // 2)
            y = _dot(_upk(h_sc[0:TM0 // 2, ks]), wd_sc[ks, _tile(NT - 1)], NN_DIMS)
            acc['y', NT - 1] = y if half == 0 else acc['y', NT - 1] + y
            return y

        def down(q, k):
            m = acc[q]
            m[k] = _dot(*out_ops(HT, q, NKH, None)[k](), NN_DIMS)
            if len(m) == 7:
                acc['y', 2 * q], acc['y', 2 * q + 1] = _ocomb(m)
            return m[k]

        def oproj(n):
            if n == 0:
                halo(TM0)
                acc['a'] = a_sc[0:TM0, :]
            y = _dot(acc['a'], _upk(wo_sc[0:D // 2, _tile(n)]), NN_DIMS, 4 if n == NT - 1 else 1)
            emit_out(0, n, acc['y', n] + y)
            return y

        units = (b.GU([10, 11]) + [(wt_sc, part(b.gu12, m)) for m in 'gu'] + b.T([2]) + b.P(range(10, 15))
                 + [(wd_sc, part(down_last, half)) for half in range(2)]
                 + [(wd_sc if k in (2, 5) else ds_sc, part(down, q, k))
                    for q in range(2) for k in (4, 5, 1, 7, 2, 3, 6)]
                 + [(wo_sc, part(oproj, n)) for n in range(NT)])
        when = [(-1, 2), (-1, 3), (1, 4), (2, 5), (3, 6)]
        pieces = [(su, 0, part(before, wqkv_raw), part(perm_vo, t), du) for t, (su, du) in enumerate(when)]
        pieces += tiny(dc(range(NKH)), 4, 14)
        pieces += tiny(wc([17, 18]), 5, 32, 32)
        pieces += tiny(dc([NKH, NKH + 1]), 7, 32, 32)
        pieces += tiny(hc([5, 6]), 9, 14, 32)
        pieces += tiny(wc([4, 5]), 11, 32, 32)
        pieces += tiny(wc([19]), 13, 32)
        pieces += ln_pieces(TM0 + z16, [(u, r) for u in (26, 27) for r in range(0, HT, 64)]
                            + [(u, r) for u in (28, 29) for r in range(0, TM0, 64)], 3)
        pieces += attn_pieces([(u, r) for u in range(11, 14) for r in range(0, TM0, 128)]
                              + [(u, r) for u in range(14, 25) for r in range(0, HT, 128)], True)
        run(units, pieces)
        wait('x3')

    @pl.when(i > 0)
    def _():
        row0 = pl.multiple_of(TM0 + (i - 1) * TM, 16)
        nxt = pl.multiple_of(jnp.minimum(row0 + TM, S - TM), 16)
        b = Block(TM)
        units = [u for p in range(7) for u in b.S(p)] + b.P([14])
        nq = len(units)
        units += [u for p in range(7, len(PAIRS)) for u in b.S(p)] + b.T([2])
        nf = len(units)
        st = {0: {}, 1: {}}

        def last_tile(half):
            if half == 0:
                halo(TM)
                st['a'] = a_sc[0:TM, :]
                kts = list(range(NCH + 1, 2 * NKP + 1)) + list(range(4))
            else:
                kts = list(range(4, NCH + 1))
            lhs = jnp.concatenate([_upk(h_sc[0:TM // 2, _tile(k)]) if k <= NCH else st['a'][:, _tile(k - NCH - 1)]
                                   for k in kts], axis=1)
            y = _dot(lhs, jnp.concatenate([orows(k, NT - 1) for k in kts], axis=0), NN_DIMS)
            if half == 0:
                st['y'] = y
            else:
                emit_out(row0, NT - 1, st['y'] + y)
            return y

        def prod(q, k):
            m = st[q]
            m[k] = _dot(*out_ops(HM, q, NKP, st['a'])[k](), NN_DIMS)
            if k == 2:
                emit_out(row0 + HM, 2 * q, (m[8][HM:TM] + m[4]) + m[2])
            elif k == 5:
                emit_out(row0, 2 * q + 1, (m[9][0:HM] + m[3]) + m[5])
            elif k == 7:
                emit_out(row0, 2 * q, ((m[8][0:HM] + m[4]) - m[5]) + (m[1] + m[7]))
            elif k == 6:
                c = (((m[9][HM:TM] + m[3]) - m[2]) + m[1]) + m[6]
                emit_out(row0 + HM, 2 * q + 1, c[0:HM - 64])
                emit_out(row0 + TM - 64, 2 * q + 1, c[HM - 64:HM])
            return m[k]

        units += [(wd_sc, part(last_tile, 0)), (wd_sc, part(last_tile, 1))]
        units += [(ds_sc, part(prod, q, k)) for q, k in
                  [(0, 4), (0, 3), (1, 4), (1, 3)] + [(q, k) for q in range(2) for k in (8, 9, 2, 5, 1, 7, 6)]]
        pieces = ln_pieces(nxt, [(4 + 2 * j, 0) for j in range(TM // LR)], 8)
        pieces += attn_pieces([(u, 0) for u in range(nq - 1, nf - 3)], False)
        slots = ([(u, r) for u in range(nf, nf + 2) for r in range(0, TM, 32)]
                 + [(u, r) for u in range(nf + 2, nf + 5) for r in range(0, HM, 32)])
        todo = [(kp, r0) for kp in range(NKH) for r0 in range(0, HM, 32)]
        pieces += [(u, r, part(before, h2_sc), part(hcomb, HM, kp, r0, 32), None) for (u, r), (kp, r0) in zip(slots, todo)]
        run(units, pieces)

    @pl.when(i == NB - 1)
    def _():
        pltpu.make_async_copy(o_sc, o_hbm, osem).wait()


@jax.jit
def pallas_parallel_sum__sliding_local_dilated__geglu_ffn__prompt_kernel(
    A_x: jax.Array,
    A_wqkv: jax.Array,
    A_wo: jax.Array,
    B_x: jax.Array,
    B_w_gate: jax.Array,
    B_w_up: jax.Array,
    B_w_down: jax.Array,
):
    assert A_x.shape == (1, S, D) and B_w_gate.shape == (D, F)
    hbm = pl.BlockSpec(memory_space=pl.ANY)
    out = pl.pallas_call(
        _kernel,
        grid=(NB,),
        in_specs=[hbm] * 6,
        out_specs=hbm,
        out_shape=jax.ShapeDtypeStruct((S, D), A_x.dtype),
        scratch_shapes=[
            pltpu.VMEM((S + 16, D), bf16),
            pltpu.VMEM((TMX // 2, D), u32),
            pltpu.VMEM((HM // 2, 5 * KS), u32),
            pltpu.VMEM((len(PAIRS) * 5 * 64 + 16, KS), u32),
            pltpu.VMEM((TMX // 4, 5 * KD), u32),
            pltpu.VMEM((5 * KD // 2 + 16, 256), u32),
            pltpu.VMEM((NT + 1, TMX, 128), f32),
            pltpu.VMEM((2 * NT, TMX + HALO, 128), f32),
            pltpu.VMEM((TMX + 16, D), bf16),
            pltpu.VMEM((TMX // 2, FP), u32),
            pltpu.VMEM((TMX // 2 + 16, FP), u32),
            pltpu.VMEM((S, D), bf16),
            pltpu.VMEM((12 * FC + 16, D), bf16),
            pltpu.VMEM((12 * FC + 16, D), bf16),
            pltpu.VMEM((3 * 128 + 16, D), bf16),
            pltpu.VMEM((D // 2 + 16, D), u32),
            pltpu.VMEM((FP + 16, D), bf16),
            pltpu.VMEM((D + 16, 3 * D), bf16),
            pltpu.VMEM((D // 2 + 16, D), u32),
            pltpu.VMEM((D // 2 + 16, D), u32),
            pltpu.VMEM((D // 2 + 16, D), u32),
            pltpu.VMEM((D, D), bf16),
            pltpu.VMEM((2, D + 32, 128), u32),
            pltpu.SemaphoreType.DMA((24,)),
            pltpu.SemaphoreType.DMA(()),
        ],
        compiler_params=pltpu.CompilerParams(
            dimension_semantics=("arbitrary",),
            vmem_limit_bytes=100 * 1024 * 1024,
            disable_semaphore_checks=True,
            disable_bounds_checks=True,
        ),
    )(A_x.reshape(S, D), A_wqkv, A_wo, B_w_gate.T, B_w_up.T, B_w_down)
    return out.reshape(1, S, D)
```
